```python
import os as _os
_os.environ.setdefault("JAX_PLATFORMS", "cpu")
import jax
import jax.numpy as jnp

def _softmax(x, axis=-1):
    return jax.nn.softmax(x, axis=axis)
def _gelu(x):
    return jax.nn.gelu(x, approximate=True)
def _silu(x):
    return jax.nn.silu(x)
def _sigmoid(x):
    return jax.nn.sigmoid(x)
def _layernorm(x, axis=-1, eps=1e-5):
    m = jnp.mean(x, axis=axis, keepdims=True)
    v = jnp.var(x, axis=axis, keepdims=True)
    return (x - m) / jnp.sqrt(v + eps)
def _scatter_add(tgt, idx, src, axis=0):
    return tgt.at[idx].add(src)
def _segment_sum(src, seg, n):
    return jax.ops.segment_sum(src, seg, n)
class _Rng:
    def __init__(self, key):
        self._k = key
    def _next(self):
        self._k, sub = jax.random.split(self._k)
        return sub
    def normal(self, shape):
        return jax.random.normal(self._next(), shape, dtype=jnp.bfloat16)
    def randint(self, lo, hi, shape):
        return jax.random.randint(self._next(), shape, lo, hi, dtype=jnp.int32)
    def uniform(self, shape, lo=0.0, hi=1.0):
        return jax.random.uniform(self._next(), shape, jnp.bfloat16, lo, hi)
    def permutation(self, n):
        return jax.random.permutation(self._next(), n)


kernel_name = 'concat_heads__mha_block__linear_attn_block__prompt'

def setup_inputs():
    _rng = _Rng(jax.random.key(int.from_bytes(__import__("os").urandom(4), "little")))
    _w = (lambda a: (lambda t: t.astype(jnp.bfloat16) if jnp.issubdtype(t.dtype, jnp.floating) else t)(jnp.asarray(a)))
    def _A_setup():
        B, S, D, H = 1, 2048, 1024, 32
        return {
            "x": _w((lambda *s: _rng.normal(s) * 0.2)(B, S, D)),
            "wqkv": _w((lambda *s: _rng.normal(s) * 0.2)(D, 3 * D)),
            "wo": _w((lambda *s: _rng.normal(s) * 0.05)(D, D)),
        }
    _A_in = _A_setup()

    def _B_setup():
        B, S, D = 1, 2048, 1024
        return {
            "x": _w((lambda *s: _rng.normal(s) * 0.05)(B, S, D)),
            "wqkv": _w((lambda *s: _rng.normal(s) * 1.6)(D, 3 * D)),
            "wo": _w((lambda *s: _rng.normal(s) * 0.1)(D, D)),
        }
    _B_in = _B_setup()

    return {
        "A_x": _A_in["x"],
        "A_wqkv": _A_in["wqkv"],
        "A_wo": _A_in["wo"],
        "B_x": _B_in["x"],
        "B_wqkv": _B_in["wqkv"],
        "B_wo": _B_in["wo"],
    }

def reference(A_x, A_wqkv, A_wo, B_x, B_wqkv, B_wo):
    def _A_ref(x, wqkv, wo):
        B, S, D = x.shape
        H = 32
        Dh = D // H
        qkv = (lambda x, *d: x.transpose(*d))((x @ wqkv).reshape(B, S, 3, H, Dh), 2, 0, 3, 1, 4)
        q, k, v = qkv[0], qkv[1], qkv[2]
        scores = jnp.einsum("bhqd,bhkd->bhqk", q, k) * (Dh ** -0.5)
        p = _softmax(scores, axis=-1)
        o = jnp.einsum("bhqk,bhkd->bhqd", p, v)
        return (lambda x, *d: x.transpose(*d))(o, 0, 2, 1, 3).reshape(B, S, D) @ wo

    def _B_ref(x, wqkv, wo):
        B, S, D = x.shape
        H = 32; Dh = D // H
        qkv = (lambda x, *d: x.transpose(*d))((x @ wqkv).reshape(B, S, 3, H, Dh), 2, 0, 3, 1, 4)
        q, k, v = qkv[0], qkv[1], qkv[2]
        phi = lambda t: jnp.where(t > 0, t + 1, jnp.exp(t)) + 1e-6
        pq, pk = phi(q), phi(k)
        kv = jnp.einsum("bhsd,bhse->bhde", pk, v)
        z = jnp.einsum("bhsd->bhd", pk)
        num = jnp.einsum("bhqd,bhde->bhqe", pq, kv)
        den = jnp.einsum("bhqd,bhd->bhq", pq, z)[..., None] + 1e-6
        o = num / den
        return (lambda x, *d: x.transpose(*d))(o, 0, 2, 1, 3).reshape(B, S, D) @ wo

    a = _A_ref(A_x, A_wqkv, A_wo)
    b = _B_ref(B_x, B_wqkv, B_wo)
    return jnp.concatenate([a, b], axis=-1)
```

```python
import contextlib
import math

import jax
import jax.numpy as jnp
from jax import lax
import jax.experimental.pallas as pl
import jax.experimental.pallas.tpu as pltpu

S = 2048
D = 1024
H = 32
DH = D // H
G = D // 128
RB = 512
NR = S // RB
QB = 256
NS = S // QB
KC = 128
NC = S // KC
SL = 32
WC = 256
NW = D // WC
U = 2
OUT_CUTS = (0, 5, 7, 8)
SCOPES = False

BF = jnp.bfloat16
F32 = jnp.float32
I32 = jnp.int32

NN = (((1,), (0,)), ((), ()))
TT = (((0,), (1,)), ((), ()))
TN = (((0,), (0,)), ((), ()))


def _scope(name):
    return jax.named_scope(name) if SCOPES else contextlib.nullcontext()


def _dot(a, b, dims=NN):
    return lax.dot_general(a, b, dims, preferred_element_type=F32)


def _phi(t):
    return jnp.where(t > 0, t + 1.0, jnp.exp(t)) + 1e-6


def _kernel(ax_hbm, aw_hbm, awo_hbm, bx_hbm, bw_hbm, bwo_hbm, out_hbm,
            ax, aw, awo, bx, bw, bwo,
            qt, kk, vt, ot, s_s, m_s, acc_s, l_s,
            pqt, t_s, zr_s, z_s, wp, obuf, in_sem, out_sem):
    def rows(r):
        if isinstance(r, int):
            return pl.ds(r * RB, RB)
        return pl.ds(pl.multiple_of(r * RB, RB), RB)

    sem_ids = iter(range(in_sem.shape[0]))

    def copy(hbm, buf, *idx):
        return pltpu.make_async_copy(hbm.at[idx], buf.at[idx], in_sem.at[next(sem_ids)])

    def start_at(r, later):
        for rr, cps in later.items():
            @pl.when(r == rr)
            def _():
                for cp in cps:
                    cp.start()

    full = slice(None)
    cp_bx = [copy(bx_hbm, bx, rows(r)) for r in range(NR)]
    cp_bk = [copy(bw_hbm, bw, full, pl.ds(D + c * WC, WC)) for c in range(NW)]
    cp_bq = copy(bw_hbm, bw, full, pl.ds(0, D))
    cp_bv = copy(bw_hbm, bw, full, pl.ds(2 * D, D))
    cp_ax = copy(ax_hbm, ax, full)
    cp_aq = copy(aw_hbm, aw, full, pl.ds(0, D))
    cp_akv = copy(aw_hbm, aw, full, pl.ds(D, 2 * D))
    cp_bwo = copy(bwo_hbm, bwo, full)
    cp_awo = copy(awo_hbm, awo, full)

    cp_bx[0].start()
    cp_bk[0].start()
    acc_s[...] = jnp.zeros(acc_s.shape, F32)
    l_s[...] = jnp.ones(l_s.shape, F32)
    for c in range(1, NW):
        cp_bk[c].start()

    def b_keys(r, pk):
        zp = jnp.sum(pk.reshape(RB // 8, 8, D), axis=0)
        tp = _dot(pk.astype(BF), bx[rows(r), :], TN)
        if isinstance(r, int):
            zr_s[...] = zp
            t_s[...] = tp
        else:
            zr_s[...] += zp
            t_s[...] += tp

    with _scope("p_b0"):
        cp_bx[0].wait()
        parts = []
        for c in range(NW):
            cp_bk[c].wait()
            if c == NW - 1:
                for r in range(1, NR):
                    cp_bx[r].start()
            parts.append(_phi(_dot(bx[rows(0), :], bw[:, D + c * WC:D + (c + 1) * WC])))
        b_keys(0, jnp.concatenate(parts, axis=1))
        for r in range(1, NR):
            cp_bx[r].wait()

    def b_loop(r, carry):
        start_at(r, {2: [cp_bv, cp_bwo, cp_ax], 3: [cp_bq, cp_akv]})
        b_keys(r, _phi(_dot(bx[rows(r), :], bw[:, D:2 * D])))
        return carry

    with _scope("p_b1"):
        lax.fori_loop(1, NR, b_loop, 0)

    with _scope("p_w"):
        cp_bv.wait()
        cp_bwo.wait()
        ri = lax.broadcasted_iota(I32, (128, 128), 0) // DH
        ci = lax.broadcasted_iota(I32, (128, 128), 1) // DH
        kvb = []
        for g in range(G):
            gs = slice(g * 128, (g + 1) * 128)
            kv = _dot(t_s[gs, :].astype(BF), bw[:, 2 * D + g * 128:2 * D + (g + 1) * 128])
            kvb.append(jnp.where(ri == ci, kv, 0.0).astype(BF))
        for g in range(G):
            gs = slice(g * 128, (g + 1) * 128)
            wp[gs, :] = _dot(kvb[g], bwo[gs, :]).astype(BF)
        zrow = jnp.sum(zr_s[...], axis=0, keepdims=True)
        z_s[...] = jnp.broadcast_to(zrow, (128, D)).T

    cp_ax.wait()
    cp_bq.wait()
    cp_akv.wait()

    def kv_loop(r, carry):
        start_at(r, {1: [cp_aq, cp_awo]})
        xr = ax[rows(r), :]
        k = _dot(xr, aw[:, D:2 * D]).astype(BF)
        for g in range(G):
            kk[g, rows(r), :] = k[:, g * 128:(g + 1) * 128]
        pq = _phi(_dot(bw[:, 0:D], bx[rows(r), :], TT))
        z = z_s[...]
        for t in range(RB // 128):
            pqh = pq[:, t * 128:(t + 1) * 128]
            den = jnp.sum((pqh * z).reshape(H, DH, 128), axis=1, keepdims=True) + 1e-6
            pqn = pqh.reshape(H, DH, 128) * (1.0 / den)
            pqt[:, pl.ds(pl.multiple_of(r * RB + t * 128, 128), 128)] = pqn.reshape(D, 128).astype(BF)
        vt[:, rows(r)] = _dot(aw[:, 2 * D:3 * D], xr, TT).astype(BF)
        return carry

    with _scope("p_a"):
        lax.fori_loop(0, NR, kv_loop, 0)

    cp_aq.wait()
    qscale = DH ** -0.5 * math.log2(math.e)

    def q_loop(r, carry):
        qt[:, rows(r)] = (_dot(aw[:, 0:D], ax[rows(r), :], TT) * qscale).astype(BF)
        obuf[rows(r), D:2 * D] = _dot(pqt[:, rows(r)], wp[...], TN).astype(BF)
        return carry

    with _scope("p_a2"):
        lax.fori_loop(0, NR, q_loop, 0)

    def out_copy(lo, n, half, sem):
        idx = (pl.ds(lo, n), pl.ds(half * D, D))
        return pltpu.make_async_copy(obuf.at[idx], out_hbm.at[idx], out_sem.at[sem])

    def masked_q(h, j):
        g = h // 4
        qg = qt[pl.ds(pl.multiple_of(g * 128, 128), 128), j * QB:(j + 1) * QB]
        return jnp.concatenate(
            [jnp.where(h % 4 == t, qg[t * DH:(t + 1) * DH], jnp.zeros((DH, QB), BF)) for t in range(4)],
            axis=0)

    def score_chunk(g, qm, j, c, mx):
        s = _dot(kk[g, c * KC:(c + 1) * KC, :], qm)
        s_s[j, c] = s
        cm = jnp.max(s.reshape(KC // 8, 8, QB), axis=0)
        return cm if mx is None else jnp.maximum(mx, cm)

    def prob_chunk(j, c, m, nl):
        slabs = []
        for r0 in reversed(range(0, KC, SL)):
            p = jnp.exp2(s_s[j, c, r0:r0 + SL, :].reshape(SL // 8, 8, QB) - m[None])
            ps = jnp.sum(p, axis=0)
            nl = -ps if nl is None else nl - ps
            pb = pltpu.bitcast(p.reshape(SL, QB).astype(BF), I32)
            pb = jnp.concatenate([pb[:-8], jnp.maximum(pb[-8:], pltpu.bitcast(nl, I32))], axis=0)
            slabs.insert(0, pltpu.bitcast(pb, BF))
        return jnp.concatenate(slabs, axis=0), nl

    def head_rows(h):
        if isinstance(h, int):
            return pl.ds(h * DH, DH)
        return pl.ds(pl.multiple_of(h * DH, DH), DH)

    def finish(h, j, acc, nl):
        o = acc * (-1.0 / jnp.sum(nl, axis=0, keepdims=True))
        ot[head_rows(h), j * QB:(j + 1) * QB] = o.astype(BF)

    def sub_block(h, j, with_next, hook=None):
        m = jnp.broadcast_to(jnp.max(m_s[j], axis=0, keepdims=True), (8, QB))
        if with_next:
            qm = masked_q(h + 1, j)
        mx = nl = acc = None
        for c in range(NC):
            p, nl = prob_chunk(j, c, m, nl)
            if with_next:
                mx = score_chunk((h + 1) // 4, qm, j, c, mx)
            d = _dot(vt[head_rows(h), c * KC:(c + 1) * KC], p)
            acc = d if acc is None else acc + d
            if hook is not None:
                hook(c)
        if with_next:
            m_s[j] = mx
        return acc, nl

    def attn_steps(h0, n, deferred):
        if deferred:
            finish(h0 - 1, NS - 1, acc_s[...], l_s[...])
        for u in range(n):
            for j in range(NS):
                acc, nl = sub_block(h0 + u, j, True)
                if u == n - 1 and j == NS - 1:
                    acc_s[...] = acc
                    l_s[...] = nl
                else:
                    finish(h0 + u, j, acc, nl)

    npeel = (H - 1) % U or U
    with _scope("p_qk0"):
        for j in range(NS):
            qm = masked_q(0, j)
            mx = None
            for c in range(NC):
                mx = score_chunk(0, qm, j, c, mx)
            m_s[j] = mx
        attn_steps(0, npeel, False)

    cp_outb = out_copy(0, S, 1, NS)

    def attn_loop(i, carry):
        start_at(i, {1: [cp_outb]})
        attn_steps(npeel + i * U, U, True)
        return carry

    with _scope("p_attn"):
        lax.fori_loop(0, (H - 1 - npeel) // U, attn_loop, 0)

    with _scope("p_outA"):
        cp_awo.wait()
        finish(H - 2, NS - 1, acc_s[...], l_s[...])
        cps = [cp_outb]
        finish(H - 1, 0, *sub_block(H - 1, 0, False))
        for j in range(NS):
            cols = slice(j * QB, (j + 1) * QB)
            oj = ot[:, cols].T

            def piece(c, cols=cols, oj=oj):
                if c % 2 == 1:
                    ns = slice(c // 2 * 128, (c // 2 + 1) * 128)
                    obuf[cols, ns] = _dot(oj, awo[:, ns]).astype(BF)

            if j + 1 < NS:
                finish(H - 1, j + 1, *sub_block(H - 1, j + 1, False, piece))
            else:
                for c in range(NC):
                    piece(c)
            if j + 1 in OUT_CUTS:
                lo = OUT_CUTS[OUT_CUTS.index(j + 1) - 1]
                cps.append(out_copy(lo * QB, (j + 1 - lo) * QB, 0, j))
                cps[-1].start()
    for cp in cps:
        cp.wait()


@jax.jit
def pallas_concat_heads__mha_block__linear_attn_block__prompt_kernel(
    A_x: jax.Array,
    A_wqkv: jax.Array,
    A_wo: jax.Array,
    B_x: jax.Array,
    B_wqkv: jax.Array,
    B_wo: jax.Array,
):
    hbm = pl.BlockSpec(memory_space=pl.ANY)
    out = pl.pallas_call(
        _kernel,
        out_shape=jax.ShapeDtypeStruct((S, 2 * D), BF),
        in_specs=[hbm] * 6,
        out_specs=hbm,
        scratch_shapes=[
            pltpu.VMEM((S, D), BF), pltpu.VMEM((D, 3 * D), BF), pltpu.VMEM((D, D), BF),
            pltpu.VMEM((S, D), BF), pltpu.VMEM((D, 3 * D), BF), pltpu.VMEM((D, D), BF),
            pltpu.VMEM((D, S), BF),
            pltpu.VMEM((G, S, 128), BF),
            pltpu.VMEM((D, S), BF),
            pltpu.VMEM((D, S), BF),
            pltpu.VMEM((NS, NC, KC, QB), F32),
            pltpu.VMEM((NS, 8, QB), F32),
            pltpu.VMEM((DH, QB), F32),
            pltpu.VMEM((8, QB), F32),
            pltpu.VMEM((D, S), BF),
            pltpu.VMEM((D, D), F32),
            pltpu.VMEM((8, D), F32),
            pltpu.VMEM((D, 128), F32),
            pltpu.VMEM((D, D), BF),
            pltpu.VMEM((S, 2 * D), BF),
            pltpu.SemaphoreType.DMA((NR + NW + 7,)),
            pltpu.SemaphoreType.DMA((NS + 1,)),
        ],
        compiler_params=pltpu.CompilerParams(vmem_limit_bytes=110 * 1024 * 1024),
        name="mha_linattn",
    )(A_x.reshape(S, D), A_wqkv, A_wo, B_x.reshape(S, D), B_wqkv, B_wo)
    return out.reshape(1, S, 2 * D)
```

```python
import math

import jax
import jax.numpy as jnp
from jax import lax
import jax.experimental.pallas as pl
import jax.experimental.pallas.tpu as pltpu

S = 2048
D = 1024
H = 32
DH = D // H
G = D // 128
RB = 512
NR = S // RB
QB = 256
NS = S // QB
KC = 128
NC = S // KC
SL = 32
WC = 256
NW = D // WC
U = 2
CUT = 4

BF = jnp.bfloat16
F32 = jnp.float32
I32 = jnp.int32

NN = (((1,), (0,)), ((), ()))
TT = (((0,), (1,)), ((), ()))
TN = (((0,), (0,)), ((), ()))


def _dot(a, b, dims=NN):
    return lax.dot_general(a, b, dims, preferred_element_type=F32)


def _phi(t):
    return jnp.where(t > 0, t + 1.0, jnp.exp(t)) + 1e-6


def _kernel(ax_hbm, aw_hbm, awo_hbm, bx_hbm, bw_hbm, bwo_hbm, out_hbm,
            ax, aw, awo, bx, bw, bwo,
            qt, kk, vt, ot, s_s, m_s, acc_s, l_s, qm_s,
            pqt, t_s, zr_s, z_s, wp, obuf, in_sem, out_sem):
    def rows(r):
        if isinstance(r, int):
            return pl.ds(r * RB, RB)
        return pl.ds(pl.multiple_of(r * RB, RB), RB)

    sem_ids = iter(range(in_sem.shape[0]))

    def copy(hbm, buf, *idx):
        return pltpu.make_async_copy(hbm.at[idx], buf.at[idx], in_sem.at[next(sem_ids)])

    def start_at(r, later):
        for rr, cps in later.items():
            @pl.when(r == rr)
            def _():
                for cp in cps:
                    cp.start()

    full = slice(None)
    cp_x0 = [copy(bx_hbm, bx, pl.ds(i * RB // 2, RB // 2)) for i in range(2)]
    cp_bx = {r: copy(bx_hbm, bx, rows(r)) for r in range(1, NR)}
    cp_bk = [copy(bw_hbm, bw, full, pl.ds(D + c * WC, WC)) for c in range(NW)]
    cp_bq = copy(bw_hbm, bw, full, pl.ds(0, D))
    cp_bv = copy(bw_hbm, bw, full, pl.ds(2 * D, D))
    cp_ax = copy(ax_hbm, ax, full)
    cp_aq = copy(aw_hbm, aw, full, pl.ds(0, D))
    cp_akv = copy(aw_hbm, aw, full, pl.ds(D, 2 * D))
    cp_bwo = copy(bwo_hbm, bwo, full)
    cp_awo = copy(awo_hbm, awo, full)

    cp_x0[0].start()
    cp_bk[0].start()
    cp_x0[1].start()
    cp_bk[1].start()

    def b_keys(r, pk):
        zp = jnp.sum(pk.reshape(RB // 8, 8, D), axis=0)
        tp = _dot(pk.astype(BF), bx[rows(r), :], TN)
        if isinstance(r, int):
            zr_s[...] = zp
            t_s[...] = tp
        else:
            zr_s[...] += zp
            t_s[...] += tp

    hb = RB // 2
    cp_x0[0].wait()
    cp_bk[0].wait()
    for c in range(2, NW):
        cp_bk[c].start()
    top = _phi(_dot(bx[0:hb, :], bw[:, D:D + WC]))
    cp_x0[1].wait()
    bot = _phi(_dot(bx[hb:RB, :], bw[:, D:D + WC]))
    parts = [jnp.concatenate([top, bot], axis=0)]
    cp_bk[1].wait()
    parts.append(_phi(_dot(bx[rows(0), :], bw[:, D + WC:D + 2 * WC])))
    for c in range(2, NW):
        cp_bk[c].wait()
    for r in range(1, NR):
        cp_bx[r].start()
    parts.append(_phi(_dot(bx[rows(0), :], bw[:, D + 2 * WC:2 * D])))
    b_keys(0, jnp.concatenate(parts, axis=1))
    for r in range(1, NR):
        cp_bx[r].wait()

    def b_loop(r, carry):
        start_at(r, {2: [cp_bv, cp_bwo, cp_ax], 3: [cp_bq, cp_akv, cp_aq]})
        b_keys(r, _phi(_dot(bx[rows(r), :], bw[:, D:2 * D])))
        return carry

    lax.fori_loop(1, NR, b_loop, 0)

    cp_bv.wait()
    cp_bwo.wait()
    ri = lax.broadcasted_iota(I32, (128, 128), 0) // DH
    ci = lax.broadcasted_iota(I32, (128, 128), 1) // DH
    kvb = []
    for g in range(G):
        gs = slice(g * 128, (g + 1) * 128)
        kv = _dot(t_s[gs, :].astype(BF), bw[:, 2 * D + g * 128:2 * D + (g + 1) * 128])
        kvb.append(jnp.where(ri == ci, kv, 0.0).astype(BF))
    for g in range(G):
        gs = slice(g * 128, (g + 1) * 128)
        wp[gs, :] = _dot(kvb[g], bwo[gs, :]).astype(BF)
    zrow = jnp.sum(zr_s[...], axis=0, keepdims=True)
    z_s[...] = jnp.broadcast_to(zrow, (128, D)).T

    cp_ax.wait()
    cp_bq.wait()
    cp_akv.wait()

    def kv_loop(r, carry):
        xr = ax[rows(r), :]
        k = _dot(xr, aw[:, D:2 * D]).astype(BF)
        for g in range(G):
            kk[g, rows(r), :] = k[:, g * 128:(g + 1) * 128]
        pq = _phi(_dot(bw[:, 0:D], bx[rows(r), :], TT))
        z = z_s[...]
        for t in range(RB // 128):
            pqh = pq[:, t * 128:(t + 1) * 128]
            den = jnp.sum((pqh * z).reshape(H, DH, 128), axis=1, keepdims=True) + 1e-6
            pqn = pqh.reshape(H, DH, 128) * (1.0 / den)
            pqt[:, pl.ds(pl.multiple_of(r * RB + t * 128, 128), 128)] = pqn.reshape(D, 128).astype(BF)
        v = _dot(aw[:, 2 * D:3 * D], xr, TT).astype(BF)
        for t in range(RB // KC):
            vt[:, r * (RB // KC) + t] = v[:, t * KC:(t + 1) * KC].reshape(H, DH, KC)
        return carry

    lax.fori_loop(0, NR, kv_loop, 0)

    cp_aq.wait()
    qscale = DH ** -0.5 * math.log2(math.e)

    def q_loop(r, carry):
        q = (_dot(ax[rows(r), :], aw[:, 0:D]) * qscale).astype(BF).T
        for t in range(RB // 128):
            qt[:, r * (RB // 128) + t] = q[:, t * 128:(t + 1) * 128].reshape(G, 128, 128)
        obuf[rows(r), D:2 * D] = _dot(pqt[:, rows(r)], wp[...], TN).astype(BF)
        return carry

    lax.fori_loop(0, NR, q_loop, 0)

    def out_copy(idx, sem):
        return pltpu.make_async_copy(obuf.at[idx], out_hbm.at[idx], out_sem.at[sem])

    def masked_q(h, j):
        qg = jnp.concatenate([qt[h // 4, j * (QB // 128) + t] for t in range(QB // 128)], axis=1)
        return jnp.concatenate(
            [jnp.where(h % 4 == t, qg[t * DH:(t + 1) * DH], jnp.zeros((DH, QB), BF)) for t in range(4)],
            axis=0)

    def score_chunk(h, j, c, qm, mx):
        s = _dot(kk[h // 4, c * KC:(c + 1) * KC, :], qm)
        s_s[j, c] = s
        for i in range(0, KC, 8):
            mx = s[i:i + 8] if mx is None else jnp.maximum(mx, s[i:i + 8])
        return mx

    def prob_chunk(j, c, m, nl):
        slabs = []
        for r0 in reversed(range(0, KC, SL)):
            p = jnp.exp2(s_s[j, c, r0:r0 + SL, :].reshape(SL // 8, 8, QB) - m[None])
            for i in reversed(range(SL // 8)):
                nl = -p[i] if nl is None else nl - p[i]
            pb = pltpu.bitcast(p.reshape(SL, QB).astype(BF), I32)
            pb = jnp.concatenate([pb[:-8], jnp.maximum(pb[-8:], pltpu.bitcast(nl, I32))], axis=0)
            slabs.insert(0, pltpu.bitcast(pb, BF))
        return jnp.concatenate(slabs, axis=0), nl

    def finish(h, j, acc, nl):
        o = acc * (-1.0 / jnp.sum(nl, axis=0, keepdims=True))
        lo = h * DH if isinstance(h, int) else pl.multiple_of(h * DH, DH)
        ot[pl.ds(lo, DH), j * QB:(j + 1) * QB] = o.astype(BF)

    def step(soft, score, qm=None, hook=None):
        mx = nl = acc = None
        if soft is not None:
            m = jnp.broadcast_to(jnp.max(m_s[soft[1]], axis=0, keepdims=True), (8, QB))
        if score is not None and qm is None:
            qm = masked_q(*score)
        for c in range(NC):
            if soft is not None:
                p, nl = prob_chunk(soft[1], c, m, nl)
            if score is not None:
                mx = score_chunk(*score, c, qm, mx)
            if soft is not None:
                d = _dot(vt[soft[0], c], p)
                acc = d if acc is None else d + acc
            if hook is not None:
                hook(c)
        if score is not None:
            m_s[score[1]] = mx
        return acc, nl

    def attn_steps(h0, n, carried):
        qm = None
        if carried:
            finish(h0, 0, acc_s[...], l_s[...])
            qm = jnp.concatenate([qm_s[t] for t in range(QB // 128)], axis=1)
        for u in range(n):
            for j in range(NS):
                soft = (h0 + u + (j + 1) // NS, (j + 1) % NS)
                acc, nl = step(soft, (h0 + u + 1, j), qm)
                qm = None
                if u == n - 1 and j == NS - 1:
                    acc_s[...] = acc
                    l_s[...] = nl
                else:
                    finish(*soft, acc, nl)
        qm = masked_q(jnp.minimum(h0 + n + 1, H - 1) if carried else h0 + n + 1, 0)
        for t in range(QB // 128):
            qm_s[t] = qm[:, t * 128:(t + 1) * 128]

    npeel = (H - 1) % U or U
    for j in range(NS - 1):
        step(None, (0, j))
    finish(0, 0, *step((0, 0), (0, NS - 1)))
    attn_steps(0, npeel, False)

    cp_outb = out_copy((pl.ds(0, S), pl.ds(D, D)), 0)

    def attn_loop(i, carry):
        start_at(i, {1: [cp_outb, cp_awo]})
        attn_steps(npeel + i * U, U, True)
        return carry

    lax.fori_loop(0, (H - 1 - npeel) // U, attn_loop, 0)

    cp_awo.wait()
    finish(H - 1, 0, acc_s[...], l_s[...])
    last = S - QB
    flush = {
        (CUT, G - 1): [out_copy((pl.ds(0, (CUT + 1) * QB), pl.ds(0, D)), 1)],
        (NS - 1, G // 2 - 1): [
            out_copy((pl.ds((CUT + 1) * QB, last - (CUT + 1) * QB), pl.ds(0, D)), 2),
            out_copy((pl.ds(last, QB), pl.ds(0, D // 2)), 3)],
        (NS - 1, G - 1): [out_copy((pl.ds(last, QB), pl.ds(D // 2, D // 2)), 4)],
    }
    for j in range(NS):
        cols = slice(j * QB, (j + 1) * QB)
        oj = ot[:, cols].T

        def piece(c, j=j, cols=cols, oj=oj):
            if c % 2 == 1:
                ns = slice(c // 2 * 128, (c // 2 + 1) * 128)
                obuf[cols, ns] = _dot(oj, awo[:, ns]).astype(BF)
                if c < NC - 1:
                    for cp in flush.get((j, c // 2), []):
                        cp.start()

        if j + 1 < NS:
            finish(H - 1, j + 1, *step((H - 1, j + 1), None, hook=piece))
        else:
            step(None, None, hook=piece)
        for cp in flush.get((j, G - 1), []):
            cp.start()
    cps = [cp_outb] + [cp for group in flush.values() for cp in group]
    for cp in cps:
        cp.wait()


@jax.jit
def pallas_concat_heads__mha_block__linear_attn_block__prompt_kernel(
    A_x: jax.Array,
    A_wqkv: jax.Array,
    A_wo: jax.Array,
    B_x: jax.Array,
    B_wqkv: jax.Array,
    B_wo: jax.Array,
):
    hbm = pl.BlockSpec(memory_space=pl.ANY)
    out = pl.pallas_call(
        _kernel,
        out_shape=jax.ShapeDtypeStruct((S, 2 * D), BF),
        in_specs=[hbm] * 6,
        out_specs=hbm,
        scratch_shapes=[
            pltpu.VMEM((S, D), BF), pltpu.VMEM((D, 3 * D), BF), pltpu.VMEM((D, D), BF),
            pltpu.VMEM((S, D), BF), pltpu.VMEM((D, 3 * D), BF), pltpu.VMEM((D, D), BF),
            pltpu.VMEM((G, S // 128, 128, 128), BF),
            pltpu.VMEM((G, S, 128), BF),
            pltpu.VMEM((H, NC, DH, KC), BF),
            pltpu.VMEM((D, S), BF),
            pltpu.VMEM((NS, NC, KC, QB), F32),
            pltpu.VMEM((NS, 8, QB), F32),
            pltpu.VMEM((DH, QB), F32),
            pltpu.VMEM((8, QB), F32),
            pltpu.VMEM((QB // 128, 128, 128), BF),
            pltpu.VMEM((D, S), BF),
            pltpu.VMEM((D, D), F32),
            pltpu.VMEM((8, D), F32),
            pltpu.VMEM((D, 128), F32),
            pltpu.VMEM((D, D), BF),
            pltpu.VMEM((S, 2 * D), BF),
            pltpu.SemaphoreType.DMA((NR + NW + 8,)),
            pltpu.SemaphoreType.DMA((5,)),
        ],
        compiler_params=pltpu.CompilerParams(vmem_limit_bytes=110 * 1024 * 1024),
        name="mha_linattn",
    )(A_x.reshape(S, D), A_wqkv, A_wo, B_x.reshape(S, D), B_wqkv, B_wo)
    return out.reshape(1, S, 2 * D)
```
